```python
import jax
import jax.numpy as jnp

def _softmax(x, axis=-1):
    return jax.nn.softmax(x, axis=axis)
def _gelu(x):
    return jax.nn.gelu(x, approximate=True)
def _silu(x):
    return jax.nn.silu(x)
def _sigmoid(x):
    return jax.nn.sigmoid(x)
def _layernorm(x, axis=-1, eps=1e-5):
    m = jnp.mean(x, axis=axis, keepdims=True)
    v = jnp.var(x, axis=axis, keepdims=True)
    return (x - m) / jnp.sqrt(v + eps)
def _scatter_add(tgt, idx, src, axis=0):
    return tgt.at[idx].add(src)
def _segment_sum(src, seg, n):
    return jax.ops.segment_sum(src, seg, n)
class _Rng:
    def __init__(self, key):
        self._k = key
    def _next(self):
        self._k, sub = jax.random.split(self._k)
        return sub
    def normal(self, shape):
        return jax.random.normal(self._next(), shape, dtype=jnp.bfloat16)
    def randint(self, lo, hi, shape):
        return jax.random.randint(self._next(), shape, lo, hi, dtype=jnp.int32)
    def uniform(self, shape, lo=0.0, hi=1.0):
        return jax.random.uniform(self._next(), shape, jnp.bfloat16, lo, hi)
    def permutation(self, n):
        return jax.random.permutation(self._next(), n)


kernel_name = 'sequential_preLN__grouped_kv_mqa__glu_gated_swiglu__prompt'

def _fwd_setup_inputs():
    _rng = _Rng(jax.random.key(int.from_bytes(__import__("os").urandom(4), "little")))
    _w = (lambda a: (lambda t: t.astype(jnp.bfloat16) if jnp.issubdtype(t.dtype, jnp.floating) else t)(jnp.asarray(a)))
    def _A_setup():
        B, S, D, H = 1, 2048, 512, 32
        Dh = D // H
        return {
            "x": _w((lambda *s: _rng.normal(s) * 0.05)(B, S, D)),
            "wq": _w((lambda *s: _rng.normal(s) * 0.05)(D, H * Dh)),
            "wk": _w((lambda *s: _rng.normal(s) * 0.05)(D, Dh)),
            "wv": _w((lambda *s: _rng.normal(s) * 0.05)(D, Dh)),
            "wo": _w((lambda *s: _rng.normal(s) * 0.05)(H * Dh, D)),
        }
    _A_in = _A_setup()

    def _B_setup():
        B, S, D, F = 1, 2048, 512, 1376
        return {
            "x": _w((lambda *s: _rng.normal(s) * 0.05)(B, S, D)),
            "w1": _w((lambda *s: _rng.normal(s) * 0.05)(D, F) * (2.0 / D) ** 0.5),
            "w3": _w((lambda *s: _rng.normal(s) * 0.05)(D, F) * (2.0 / D) ** 0.5),
            "w2": _w((lambda *s: _rng.normal(s) * 0.05)(F, D) * (2.0 / F) ** 0.5),
        }
    _B_in = _B_setup()

    return {
        "A_x": _A_in["x"],
        "A_wq": _A_in["wq"],
        "A_wk": _A_in["wk"],
        "A_wv": _A_in["wv"],
        "A_wo": _A_in["wo"],
        "B_x": _B_in["x"],
        "B_w1": _B_in["w1"],
        "B_w3": _B_in["w3"],
        "B_w2": _B_in["w2"],
    }

def _fwd_reference(A_x, A_wq, A_wk, A_wv, A_wo, B_x, B_w1, B_w3, B_w2):
    def _A_ref(x, wq, wk, wv, wo):
        B, S, D = x.shape
        H = 32
        Dh = D // H
        q = (lambda x, *d: x.transpose(*d))((x @ wq).reshape(B, S, H, Dh), 0, 2, 1, 3)
        k = x @ wk
        v = x @ wv
        scores = jnp.einsum("bhqd,bkd->bhqk", q, k) * (Dh ** -0.5)
        p = _softmax(scores, axis=-1)
        o = jnp.einsum("bhqk,bkd->bhqd", p, v)
        return (lambda x, *d: x.transpose(*d))(o, 0, 2, 1, 3).reshape(B, S, H * Dh) @ wo

    def _B_ref(x, w1, w3, w2):
        gate = jnp.einsum("bsd,df->bsf", x, w1)
        up = jnp.einsum("bsd,df->bsf", x, w3)
        h = _silu(gate) * up
        out = jnp.einsum("bsf,fd->bsd", h, w2)
        return out

    x = A_x
    h = x + _A_ref(_layernorm(x, axis=-1), A_wq, A_wk, A_wv, A_wo)
    h2 = h + _B_ref(_layernorm(h, axis=-1), B_w1, B_w3, B_w2)
    return h2


def setup_inputs():
    _inp = _fwd_setup_inputs()
    _gk = jax.random.fold_in(jax.random.key(int.from_bytes(__import__("os").urandom(4), "little")), 2**31 - 1)
    _shapes = [[1, 2048, 512]]
    _dtypes = ['bfloat16']
    _gks = jax.random.split(_gk, len(_shapes))
    _gs = [jax.random.normal(k, s, dtype=jnp.dtype(d)) * 0.05 for k, s, d in zip(_gks, _shapes, _dtypes)]
    _inp["grad_out"] = _gs[0]
    return _inp

def reference(A_x, A_wq, A_wk, A_wv, A_wo, B_w1, B_w3, B_w2, B_x, grad_out):
    _const = dict(B_x=B_x)
    def _f(*_d):
        return _fwd_reference(**{'A_x': _d[0], 'A_wq': _d[1], 'A_wk': _d[2], 'A_wv': _d[3], 'A_wo': _d[4], 'B_w1': _d[5], 'B_w3': _d[6], 'B_w2': _d[7], **_const})
    _out, _vjp = jax.vjp(_f, A_x, A_wq, A_wk, A_wv, A_wo, B_w1, B_w3, B_w2)
    _grads = _vjp(grad_out)
    _out0 = jnp.asarray(_out)
    return (_out0, *[jnp.asarray(_g) for _g in _grads])
```

```python
import math

import jax
import jax.numpy as jnp
from jax import lax
import jax.experimental.pallas as pl
import jax.experimental.pallas.tpu as pltpu

S = 2048
D = 512
H = 32
DH = 16
F = 1376
BQ = 256
NB = S // BQ
W = 128
NJ = BQ // W

EPS = 1e-5
LOG2E = math.log2(math.e)
LN2 = math.log(2.0)
QSCALE = (DH ** -0.5) * LOG2E
SAFE_L = 2.0 ** -40

f32 = jnp.float32
bf16 = jnp.bfloat16
NT = (((1,), (1,)), ((), ()))

FWD_KC, FWD_U, FWD_L, BWD_KC, BWD_U, BWD_L = 256, 4, 6, 128, 4, 8


def _dot(a, b):
    return jnp.dot(a, b, preferred_element_type=f32)


def _dot_nt(a, b):
    return lax.dot_general(a, b, NT, preferred_element_type=f32)


def _bf(x):
    return pltpu.bitcast(x, bf16)


def _tr(x):
    return x.astype(f32).T.astype(bf16)


def _lnT_fwd(x):
    m = jnp.mean(x, axis=0, keepdims=True)
    xc = x - m
    v = jnp.mean(xc * xc, axis=0, keepdims=True)
    rstd = lax.rsqrt(v + EPS)
    return xc * rstd, rstd


def _lnT_bwd(dy, xhat, rstd):
    m1 = jnp.mean(dy, axis=0, keepdims=True)
    m2 = jnp.mean(dy * xhat, axis=0, keepdims=True)
    return rstd * (dy - m1 - xhat * m2)


def _split3_rows(val, n, lanes):
    hi = val.astype(bf16).astype(f32)
    r1 = val - hi
    mid = r1.astype(bf16).astype(f32)
    lo = (r1 - mid).astype(bf16).astype(f32)
    row = lax.broadcasted_iota(jnp.int32, (n, 16, lanes), 1)
    zero = jnp.zeros((n, 16, lanes), f32)
    return jnp.where(row == 0, hi, jnp.where(row == 1, mid, jnp.where(row == 2, lo, zero)))


def _kernel(x_hbm, wq_hbm, wkT_hbm, wvT_hbm, wo_hbm, w1T_hbm, w3T_hbm, w2_hbm, g_ref,
            out_ref, dx_hbm, dwq_hbm, dwkT_hbm, dwvT_hbm, dwo_hbm, dw1T_hbm, dw3T_hbm, dw2_hbm,
            x_ref, wq_ref, wkv_ref, wo_ref, w1T_ref, w3T_ref, w2_ref, dwkv_s, in_sem, out_sem,
            xT_s, xnT_s, wqT_s, woT_s, w1_s, w3_s, w2T_s, ka_s, va_s, kT_s, vT_s, kmax_s,
            qa_s, doa_s, p_s, oT_s, l_s, dqT_s, dkT_s, dvT_s,
            dhT_s, dxnT_s, a_wq, a_wo, a_w1T, a_w3T, a_w2, flag_s):
    i = pl.program_id(0)

    ka32 = ka_s.bitcast(jnp.uint32)
    va32 = va_s.bitcast(jnp.uint32)
    kT32 = kT_s.bitcast(jnp.uint32)
    vT32 = vT_s.bitcast(jnp.uint32)
    qa32 = qa_s.bitcast(jnp.uint32)
    doa32 = doa_s.bitcast(jnp.uint32)
    p32 = p_s.bitcast(jnp.uint32)

    def x_copy(b):
        rws = pl.ds(b * BQ, BQ)
        return pltpu.make_async_copy(x_hbm.at[rws, :], x_ref.at[rws, :], in_sem.at[b])

    wk_copy = pltpu.make_async_copy(wkT_hbm, wkv_ref.at[0:DH, :], in_sem.at[NB])
    wv_copy = pltpu.make_async_copy(wvT_hbm, wkv_ref.at[DH:2 * DH, :], in_sem.at[NB + 1])
    wq_copy = pltpu.make_async_copy(wq_hbm, wq_ref, in_sem.at[NB + 2])
    wo_copy = pltpu.make_async_copy(wo_hbm, wo_ref, in_sem.at[NB + 3])
    w1_copy = pltpu.make_async_copy(w1T_hbm, w1T_ref, in_sem.at[NB + 4])
    w3_copy = pltpu.make_async_copy(w3T_hbm, w3T_ref, in_sem.at[NB + 5])
    w2_copy = pltpu.make_async_copy(w2_hbm, w2_ref, in_sem.at[NB + 6])

    @pl.when(i == 0)
    def _prologue():
        wk_copy.start()
        wv_copy.start()
        for b in range(NB):
            x_copy(b).start()
        wq_copy.start()
        wk_copy.wait()
        wv_copy.wait()
        wkvT = wkv_ref[...]
        row = lax.broadcasted_iota(jnp.int32, (128, BQ), 0)
        lane = lax.broadcasted_iota(jnp.int32, (BQ, 32), 1)

        kmax = jnp.zeros((1, BQ), f32)
        for b in range(NB):
            cols = pl.ds(b * BQ, BQ)
            x_copy(b).wait()
            xT = x_ref[cols, :].astype(f32).T
            xT_s[:, cols] = xT.astype(bf16)
            xhat, _ = _lnT_fwd(xT)
            xnT = xhat.astype(bf16)
            xnT_s[:, cols] = xnT
            kvT = _dot(wkvT, xnT).astype(bf16).astype(f32)
            kT_s[:, cols] = kvT[0:DH].astype(bf16)
            vT_s[:, cols] = kvT[DH:2 * DH].astype(bf16)
            ones = jnp.where(row[0:DH] < 3, 1.0, 0.0).astype(f32)
            pad = jnp.zeros((128 - 2 * DH, BQ), f32)
            ka = jnp.concatenate([kvT[0:DH], ones, pad], axis=0).T
            va = jnp.concatenate([kvT[DH:2 * DH], ones, pad], axis=0).T
            ka_s[cols, :] = ka[:, 0:32].astype(bf16)
            va_s[cols, :] = va[:, 0:32].astype(bf16)
            kn = jnp.sum(kvT[0:DH] * kvT[0:DH], axis=0, keepdims=True)
            kmax = jnp.maximum(kmax, kn)
            if b == NB // 2:
                wo_copy.start()
                w1_copy.start()
                w3_copy.start()
                w2_copy.start()

        kmax = jnp.sqrt(jnp.max(kmax, axis=1, keepdims=True))
        kmax_s[...] = jnp.broadcast_to(kmax, kmax_s.shape)
        dkT_s[...] = jnp.zeros_like(dkT_s)
        dvT_s[...] = jnp.zeros_like(dvT_s)
        wq_copy.wait()
        wqT_s[...] = _tr(wq_ref[...])

    cols = pl.ds(pl.multiple_of(i * BQ, BQ), BQ)
    xnT = xnT_s[:, cols]

    with jax.named_scope("qproj"):
        qT = (_dot(wqT_s[...], xnT) * QSCALE).astype(bf16).astype(f32)
        q3 = qT.reshape(H, DH, BQ)
        qn = jnp.sqrt(jnp.sum(q3 * q3, axis=1, keepdims=True))
        mhat = qn * kmax_s[0:1, :] * (1.0 + 2.0 ** -10)
        qa = jnp.concatenate([q3, _split3_rows(-mhat, H, BQ)], axis=1).reshape(2 * D, BQ).astype(bf16)
        for j in range(NJ):
            qa_s[j] = qa[:, j * W:(j + 1) * W]

    def fwd_group(gi, carry):
        kc, U, L = FWD_KC, FWD_U, FWD_L
        nc = S // kc
        h0 = gi * U
        pr = p32.at[pl.ds(h0, U)]
        pbr = p_s.at[pl.ds(h0, U)]
        items = [(u, j, c) for u in range(U) for j in range(NJ) for c in range(nc)]
        n = len(items)
        acc, lsum = {}, {}

        def r0(u):
            return pl.multiple_of((h0 + u) * 16, 16)

        def a_part(t):
            u, j, c = items[t]
            qh = _bf(qa32[j, pl.ds(r0(u), 16), :])
            s = _dot(_bf(ka32[c * kc // 2:(c + 1) * kc // 2, :]), qh)
            p = jnp.exp2(s)
            t8 = jnp.sum(p.reshape(kc // 8, 8, W), axis=0)
            lsum[(u, j)] = t8 if c == 0 else lsum[(u, j)] + t8
            pbr[u, j, c * kc:(c + 1) * kc, :] = p.astype(bf16)

        def b_part(t):
            u, j, c = items[t]
            r = _dot(_bf(vT32[:, c * kc:(c + 1) * kc]), _bf(pr[u, j, c * kc // 2:(c + 1) * kc // 2, :]))
            acc[(u, j)] = r if c == 0 else acc[(u, j)] + r
            if c == nc - 1:
                l = jnp.sum(lsum[(u, j)], axis=0, keepdims=True)
                linv = 1.0 / l
                oT_s[j, pl.ds(r0(u), 16), :] = acc[(u, j)] * linv
                l_s[j, pl.ds(h0 + u, 1), :] = l

        for t in range(n + L):
            if t < n:
                a_part(t)
            if t - L >= 0:
                b_part(t - L)
        return carry

    def true_max(h, carry):
        rr = pl.multiple_of(h * 32, 32)
        for j in range(NJ):
            qh = qa_s[j, pl.ds(rr, 32), :].astype(f32)
            row = lax.broadcasted_iota(jnp.int32, (32, W), 0)
            qh = jnp.where(row < DH, qh, 0.0).astype(bf16)
            m = None
            for c in range(S // 256):
                s = _dot(ka_s[c * 256:(c + 1) * 256, :], qh)
                mc = jnp.max(s, axis=0, keepdims=True)
                m = mc if m is None else jnp.maximum(m, mc)
            ext = _split3_rows(-m.reshape(1, 1, W), 1, W).reshape(16, W)
            qa_s[j, pl.ds(pl.multiple_of(rr + 16, 16), 16), :] = ext.astype(bf16)
        return carry

    flag_s[0] = 0

    def attempt(it, carry):
        @pl.when(jnp.logical_or(it == 0, flag_s[0] == 1))
        def _():
            @pl.when(it == 1)
            def _():
                lax.fori_loop(0, H, true_max, 0)
            lax.fori_loop(0, H // FWD_U, fwd_group, 0)
            lmin = jnp.min(jnp.minimum(l_s[0], l_s[1]))
            flag_s[0] = jnp.where(lmin >= SAFE_L, 0, 1).astype(jnp.int32)
        return carry

    with jax.named_scope("attn_fwd"):
        lax.fori_loop(0, 2, attempt, 0)

    @pl.when(i == 0)
    def _weights():
        wo_copy.wait()
        woT_s[...] = _tr(wo_ref[...])
        w1_copy.wait()
        w1_s[...] = _tr(w1T_ref[...])
        w3_copy.wait()
        w3_s[...] = _tr(w3T_ref[...])
        w2_copy.wait()
        w2T_s[...] = _tr(w2_ref[...])

    def acc(ref, val):
        ref[...] = jnp.where(i == 0, 0.0, ref[...]) + val

    with jax.named_scope("dense"):
        oT = jnp.concatenate([oT_s[j] for j in range(NJ)], axis=1)
        oTb = oT.astype(bf16)
        hT = xT_s[:, cols].astype(f32) + _dot(woT_s[...], oTb)
        hhat, hrstd = _lnT_fwd(hT)
        hnT = hhat.astype(bf16)
        gate = _dot(w1T_ref[...], hnT)
        up = _dot(w3T_ref[...], hnT)
        sig = jax.nn.sigmoid(gate)
        silu = gate * sig
        act = (silu * up).astype(bf16)
        out_ref[...] = (hT + _dot(w2T_s[...], act)).T.astype(out_ref.dtype)

        g = g_ref[...]
        gT = g.astype(f32).T
        dact = _dot_nt(w2_ref[...], g)
        dup = (dact * silu).astype(bf16)
        dgate = (dact * up * (sig * (1.0 + gate * (1.0 - sig)))).astype(bf16)
        acc(a_w1T, _dot_nt(dgate, hnT))
        acc(a_w3T, _dot_nt(dup, hnT))
        acc(a_w2, _dot(act, g))
        dhn = _dot(w1_s[...], dgate) + _dot(w3_s[...], dup)
        dhT = gT + _lnT_bwd(dhn, hhat, hrstd)
        dhT_s[:, cols] = dhT
        dhb = dhT.astype(bf16)
        acc(a_wo, _dot_nt(oTb, dhb))
        doT = _dot(wo_ref[...], dhb)

        linv = 1.0 / jnp.concatenate([l_s[j] for j in range(NJ)], axis=1)
        do3 = doT.reshape(H, DH, BQ)
        delta = jnp.sum(do3 * oT.reshape(H, DH, BQ), axis=1, keepdims=True)
        linv3 = linv.reshape(H, 1, BQ)
        doa = jnp.concatenate([do3 * linv3, _split3_rows(-delta * linv3, H, BQ)], axis=1)
        doa = doa.reshape(2 * D, BQ).astype(bf16)
        for j in range(NJ):
            doa_s[j] = doa[:, j * W:(j + 1) * W]

    dw1_copy = pltpu.make_async_copy(w1T_ref, dw1T_hbm, out_sem.at[0])
    dw3_copy = pltpu.make_async_copy(w3T_ref, dw3T_hbm, out_sem.at[1])
    dw2_copy = pltpu.make_async_copy(w2_ref, dw2_hbm, out_sem.at[2])
    dwo_copy = pltpu.make_async_copy(wo_ref, dwo_hbm, out_sem.at[3])

    @pl.when(i == NB - 1)
    def _early_out():
        w1T_ref[...] = a_w1T[...].astype(bf16)
        dw1_copy.start()
        w3T_ref[...] = a_w3T[...].astype(bf16)
        dw3_copy.start()
        w2_ref[...] = a_w2[...].astype(bf16)
        dw2_copy.start()
        wo_ref[...] = a_wo[...].astype(bf16)
        dwo_copy.start()

    def bwd_group(gi, carry):
        kc, U, L = BWD_KC, BWD_U, BWD_L
        nc = S // kc
        h0 = gi * U
        pr = p32.at[pl.ds(h0, U)]
        items = [(u, j, c) for u in range(U) for j in range(NJ) for c in range(nc)]
        n = len(items)
        dsv, dq = {}, {}

        def r0(u):
            return pl.multiple_of((h0 + u) * 16, 16)

        def d_part(t):
            u, j, c = items[t]
            do_aug = _bf(doa32[j, pl.ds(r0(u), 16), :])
            dp = _dot(_bf(va32[c * kc // 2:(c + 1) * kc // 2, :]), do_aug)
            pc = _bf(pr[u, j, c * kc // 2:(c + 1) * kc // 2, :])
            dsv[t] = (pc.astype(f32) * dp).astype(bf16)

        def e_part(t):
            u, j, c = items[t]
            do16 = _bf(doa32[j, pl.ds(r0(u), 8), :])
            pc = _bf(pr[u, j, c * kc // 2:(c + 1) * kc // 2, :])
            dvT_s[:, c * kc:(c + 1) * kc] += _dot_nt(do16, pc)

        def f_part(t):
            u, j, c = items[t]
            r = _dot(_bf(kT32[:, c * kc:(c + 1) * kc]), dsv[t])
            dq[(u, j)] = r if c == 0 else dq[(u, j)] + r
            if c == nc - 1:
                dqT_s[j, pl.ds(r0(u), 16), :] = dq[(u, j)]

        def g_part(t):
            u, j, c = items[t]
            q16 = _bf(qa32[j, pl.ds(r0(u), 8), :])
            dkT_s[:, c * kc:(c + 1) * kc] += _dot_nt(q16, dsv.pop(t))

        for t in range(n + L):
            if t < n:
                d_part(t)
            if t - L >= 0:
                e_part(t - L)
                f_part(t - L)
                g_part(t - L)
        return carry

    with jax.named_scope("attn_bwd"):
        lax.fori_loop(0, H // BWD_U, bwd_group, 0)

    with jax.named_scope("dq"):
        dqT = (jnp.concatenate([dqT_s[j] for j in range(NJ)], axis=1) * (DH ** -0.5)).astype(bf16)
        acc(a_wq, _dot_nt(xnT, dqT))
        dxnT_s[:, cols] = _dot(wq_ref[...], dqT)

    @pl.when(i == NB - 1)
    def _epilogue():
        wq_ref[...] = a_wq[...].astype(bf16)
        dwq_copy = pltpu.make_async_copy(wq_ref, dwq_hbm, out_sem.at[4])
        dwq_copy.start()
        wkv = jnp.concatenate([wkv_ref[...].astype(f32), jnp.zeros((128 - 2 * DH, D), f32)], axis=0)
        wkv = wkv.T[:, 0:2 * DH].astype(bf16)
        dx_copies = []
        for b in range(NB):
            cs = pl.ds(b * BQ, BQ)
            xhat, rstd = _lnT_fwd(xT_s[:, cs].astype(f32))
            dkv = jnp.concatenate([dkT_s[:, cs] * LN2, dvT_s[:, cs]], axis=0)
            dxn = dxnT_s[:, cs] + _dot(wkv, dkv.astype(bf16))
            dxT = dhT_s[:, cs] + _lnT_bwd(dxn, xhat, rstd)
            x_ref[cs, :] = dxT.T.astype(bf16)
            cp = pltpu.make_async_copy(x_ref.at[cs, :], dx_hbm.at[cs, :], out_sem.at[7 + b])
            cp.start()
            dx_copies.append(cp)
        dkvT = jnp.concatenate([dkT_s[...] * LN2, dvT_s[...]], axis=0).astype(bf16)
        dwkv_s[...] = _dot_nt(dkvT, xnT_s[...]).astype(bf16)
        dwk_copy = pltpu.make_async_copy(dwkv_s.at[0:DH, :], dwkT_hbm, out_sem.at[5])
        dwv_copy = pltpu.make_async_copy(dwkv_s.at[DH:2 * DH, :], dwvT_hbm, out_sem.at[6])
        dwk_copy.start()
        dwv_copy.start()
        dw1_copy.wait()
        dw3_copy.wait()
        dw2_copy.wait()
        dwo_copy.wait()
        dwq_copy.wait()
        for cp in dx_copies:
            cp.wait()
        dwk_copy.wait()
        dwv_copy.wait()


def _const(shape):
    nd = len(shape)
    return pl.BlockSpec(shape, lambda i: (0,) * nd, pipeline_mode=pl.Buffered(1))


@jax.jit
def pallas_sequential_preLN__grouped_kv_mqa__glu_gated_swiglu__prompt_kernel(A_x, A_wq, A_wk, A_wv, A_wo, B_x, B_w1, B_w3, B_w2, grad_out):
    del B_x
    x = A_x.reshape(S, D)
    g = grad_out.reshape(S, D)
    out_shape = [
        jax.ShapeDtypeStruct((S, D), bf16),
        jax.ShapeDtypeStruct((S, D), bf16),
        jax.ShapeDtypeStruct((D, D), bf16),
        jax.ShapeDtypeStruct((DH, D), bf16),
        jax.ShapeDtypeStruct((DH, D), bf16),
        jax.ShapeDtypeStruct((D, D), bf16),
        jax.ShapeDtypeStruct((F, D), bf16),
        jax.ShapeDtypeStruct((F, D), bf16),
        jax.ShapeDtypeStruct((F, D), bf16),
    ]
    hbm = pl.BlockSpec(memory_space=pl.ANY)
    in_specs = [hbm] * 8 + [pl.BlockSpec((BQ, D), lambda i: (i, 0))]
    out_specs = [pl.BlockSpec((BQ, D), lambda i: (i, 0))] + [hbm] * 8
    scratch = [
        pltpu.VMEM((S, D), bf16),
        pltpu.VMEM((D, D), bf16),
        pltpu.VMEM((2 * DH, D), bf16),
        pltpu.VMEM((D, D), bf16),
        pltpu.VMEM((F, D), bf16),
        pltpu.VMEM((F, D), bf16),
        pltpu.VMEM((F, D), bf16),
        pltpu.VMEM((2 * DH, D), bf16),
        pltpu.SemaphoreType.DMA((NB + 7,)),
        pltpu.SemaphoreType.DMA((NB + 7,)),
        pltpu.VMEM((D, S), bf16),
        pltpu.VMEM((D, S), bf16),
        pltpu.VMEM((D, D), bf16),
        pltpu.VMEM((D, D), bf16),
        pltpu.VMEM((D, F), bf16),
        pltpu.VMEM((D, F), bf16),
        pltpu.VMEM((D, F), bf16),
        pltpu.VMEM((S, 32), bf16),
        pltpu.VMEM((S, 32), bf16),
        pltpu.VMEM((DH, S), bf16),
        pltpu.VMEM((DH, S), bf16),
        pltpu.VMEM((8, BQ), f32),
        pltpu.VMEM((NJ, 2 * D, W), bf16),
        pltpu.VMEM((NJ, 2 * D, W), bf16),
        pltpu.VMEM((H, NJ, S, W), bf16),
        pltpu.VMEM((NJ, D, W), f32),
        pltpu.VMEM((NJ, H, W), f32),
        pltpu.VMEM((NJ, D, W), f32),
        pltpu.VMEM((DH, S), f32),
        pltpu.VMEM((DH, S), f32),
        pltpu.VMEM((D, S), f32),
        pltpu.VMEM((D, S), f32),
        pltpu.VMEM((D, D), f32),
        pltpu.VMEM((D, D), f32),
        pltpu.VMEM((F, D), f32),
        pltpu.VMEM((F, D), f32),
        pltpu.VMEM((F, D), f32),
        pltpu.SMEM((1,), jnp.int32),
    ]
    outs = pl.pallas_call(
        _kernel,
        grid=(NB,),
        in_specs=in_specs,
        out_specs=out_specs,
        out_shape=out_shape,
        scratch_shapes=scratch,
        compiler_params=pltpu.CompilerParams(
            dimension_semantics=("arbitrary",),
            vmem_limit_bytes=120 * 1024 * 1024,
        ),
    )(x, A_wq, A_wk.T, A_wv.T, A_wo, B_w1.T, B_w3.T, B_w2, g)
    h2, dx, dwq, dwkT, dwvT, dwo, dw1T, dw3T, dw2 = outs
    return (h2.reshape(1, S, D), dx.reshape(1, S, D), dwq, dwkT.T, dwvT.T, dwo, dw1T.T, dw3T.T, dw2)
```

```python
import math

import jax
import jax.numpy as jnp
from jax import lax
import jax.experimental.pallas as pl
import jax.experimental.pallas.tpu as pltpu

S = 2048
D = 512
H = 32
DH = 16
F = 1376
BQ = 256
NB = S // BQ
W = 128
NJ = BQ // W

EPS = 1e-5
LOG2E = math.log2(math.e)
LN2 = math.log(2.0)
QSCALE = (DH ** -0.5) * LOG2E
SAFE_L = 2.0 ** -64

f32 = jnp.float32
bf16 = jnp.bfloat16
NT = (((1,), (1,)), ((), ()))

FWD_KC, FWD_U, FWD_L, BWD_KC, BWD_U, BWD_LE, BWD_LF, BWD_LG, BWD_ORD = 256, 8, 10, 128, 8, 6, 8, 8, 2


def _dot(a, b):
    return jnp.dot(a, b, preferred_element_type=f32)


def _dot_nt(a, b):
    return lax.dot_general(a, b, NT, preferred_element_type=f32)


def _bf(x):
    return pltpu.bitcast(x, bf16)


def _tr(x):
    return x.T


def _lnT_fwd(x):
    m = jnp.mean(x, axis=0, keepdims=True)
    xc = x - m
    v = jnp.mean(xc * xc, axis=0, keepdims=True)
    rstd = lax.rsqrt(v + EPS)
    return xc * rstd, rstd


def _lnT_bwd(dy, xhat, rstd):
    m1 = jnp.mean(dy, axis=0, keepdims=True)
    m2 = jnp.mean(dy * xhat, axis=0, keepdims=True)
    return rstd * (dy - m1 - xhat * m2)


def _split3_rows(val, n, lanes):
    hi = val.astype(bf16).astype(f32)
    r1 = val - hi
    mid = r1.astype(bf16).astype(f32)
    lo = (r1 - mid).astype(bf16).astype(f32)
    row = lax.broadcasted_iota(jnp.int32, (n, 16, lanes), 1)
    zero = jnp.zeros((n, 16, lanes), f32)
    return jnp.where(row == 0, hi, jnp.where(row == 1, mid, jnp.where(row == 2, lo, zero)))


def _kernel(x_hbm, wq_hbm, wkT_hbm, wvT_hbm, wo_hbm, w1T_hbm, w3T_hbm, w2_hbm, g_ref,
            out_ref, dx_hbm, dwq_hbm, dwkT_hbm, dwvT_hbm, dwo_hbm, dw1T_hbm, dw3T_hbm, dw2_hbm,
            x_ref, wq_ref, wkv_ref, wo_ref, w1T_ref, w3T_ref, w2_ref, dwkv_s, in_sem, out_sem,
            rstd_s, xnT_s, wqT_s, woT_s, w1_s, w3_s, w2T_s, ka_s, va_s, kT_s, vT_s, kmax_s,
            qa_s, doa_s, p_s, p2_s, oT_s, l_s, dqT_s, dkT_s, dvT_s,
            dhT_s, dxnT_s, a_wq, a_wo, a_w1T, a_w3T, a_w2, flag_s):
    i = pl.program_id(0)

    ka32 = ka_s.bitcast(jnp.uint32)
    va32 = va_s.bitcast(jnp.uint32)
    kT32 = kT_s.bitcast(jnp.uint32)
    vT32 = vT_s.bitcast(jnp.uint32)
    qa32 = qa_s.bitcast(jnp.uint32)
    doa32 = doa_s.bitcast(jnp.uint32)
    p32 = p_s.bitcast(jnp.uint32)
    p2_32 = p2_s.bitcast(jnp.uint32)

    def x_copy(b):
        rws = pl.ds(pl.multiple_of(b * BQ, BQ), BQ)
        return pltpu.make_async_copy(x_hbm.at[rws, :], x_ref.at[rws, :], in_sem.at[b])

    wk_copy = pltpu.make_async_copy(wkT_hbm, wkv_ref.at[0:DH, :], in_sem.at[NB])
    wv_copy = pltpu.make_async_copy(wvT_hbm, wkv_ref.at[DH:2 * DH, :], in_sem.at[NB + 1])
    wq_copy = pltpu.make_async_copy(wq_hbm, wq_ref, in_sem.at[NB + 2])
    wo_copy = pltpu.make_async_copy(wo_hbm, wo_ref, in_sem.at[NB + 3])
    w1_copy = pltpu.make_async_copy(w1T_hbm, w1T_ref, in_sem.at[NB + 4])
    w3_copy = pltpu.make_async_copy(w3T_hbm, w3T_ref, in_sem.at[NB + 5])
    w2_copy = pltpu.make_async_copy(w2_hbm, w2_ref, in_sem.at[NB + 6])

    @pl.when(i == 0)
    def _prologue():
        wk_copy.start()
        wv_copy.start()
        for b in range(NB):
            x_copy(b).start()
        wq_copy.start()
        wk_copy.wait()
        wv_copy.wait()
        wkvT = wkv_ref[...]
        row = lax.broadcasted_iota(jnp.int32, (128, BQ), 0)
        lane = lax.broadcasted_iota(jnp.int32, (BQ, 32), 1)

        def blk(b, kmax):
            cols = pl.ds(pl.multiple_of(b * BQ, BQ), BQ)
            x_copy(b).wait()
            xT = x_ref[cols, :].astype(f32).T
            xhat, rstd = _lnT_fwd(xT)
            rstd_s[:, cols] = rstd
            xnT = xhat.astype(bf16)
            xnT_s[:, cols] = xnT
            kvT = _dot(wkvT, xnT).astype(bf16).astype(f32)
            kT_s[:, cols] = kvT[0:DH].astype(bf16)
            vT_s[:, cols] = kvT[DH:2 * DH].astype(bf16)
            ones = jnp.where(row[0:DH] < 3, 1.0, 0.0).astype(f32)
            pad = jnp.zeros((128 - 2 * DH, BQ), f32)
            ka = jnp.concatenate([kvT[0:DH], ones, pad], axis=0).T
            va = jnp.concatenate([kvT[DH:2 * DH], ones, pad], axis=0).T
            ka_s[cols, :] = ka[:, 0:32].astype(bf16)
            va_s[cols, :] = va[:, 0:32].astype(bf16)
            kn = jnp.sum(kvT[0:DH] * kvT[0:DH], axis=0, keepdims=True)

            @pl.when(b == 1)
            def _():
                wo_copy.start()
                w1_copy.start()
                w3_copy.start()
                w2_copy.start()
            return jnp.maximum(kmax, kn)

        kmax = lax.fori_loop(0, NB // 2, lambda b, km: blk(2 * b + 1, blk(2 * b, km)), jnp.zeros((1, BQ), f32))

        kmax = jnp.sqrt(jnp.max(kmax, axis=1, keepdims=True))
        kmax_s[...] = jnp.broadcast_to(kmax, kmax_s.shape)
        wq_copy.wait()
        wqT_s[...] = _tr(wq_ref[...])
        dkT_s[...] = jnp.zeros_like(dkT_s)
        dvT_s[...] = jnp.zeros_like(dvT_s)

    cols = pl.ds(pl.multiple_of(i * BQ, BQ), BQ)
    xnT = xnT_s[:, cols]

    qT = (_dot(wqT_s[...], xnT) * QSCALE).astype(bf16).astype(f32)
    q3 = qT.reshape(H, DH, BQ)
    qn = jnp.sqrt(jnp.sum(q3 * q3, axis=1, keepdims=True))
    mhat = qn * kmax_s[0:1, :] * (1.0 + 2.0 ** -10)
    qa = jnp.concatenate([q3, _split3_rows(-mhat, H, BQ)], axis=1).reshape(2 * D, BQ).astype(bf16)
    for j in range(NJ):
        qa_s[j] = qa[:, j * W:(j + 1) * W]

    def fwd_group(gi, carry):
        kc, U, L = FWD_KC, FWD_U, FWD_L
        nc = S // kc
        h0 = gi * U
        pr = p32.at[pl.ds(h0, U)]
        pbr = p_s.at[pl.ds(h0, U)]
        p2r = p2_s.at[pl.ds(h0, U)]
        items = [(u, j, c) for u in range(U) for j in range(NJ) for c in range(nc)]
        n = len(items)
        acc, lsum = {}, {}

        def r0(u):
            return pl.multiple_of((h0 + u) * 16, 16)

        def a_part(t):
            u, j, c = items[t]
            qh = _bf(qa32[j, pl.ds(r0(u), 16), :])
            s = _dot(_bf(ka32[c * kc // 2:(c + 1) * kc // 2, :]), qh)
            p = jnp.exp2(s)
            t8 = jnp.sum(p.reshape(kc // 8, 8, W), axis=0)
            lsum[(u, j)] = t8 if c == 0 else lsum[(u, j)] + t8
            pbr[u, j, c * kc:(c + 1) * kc, :] = p.astype(bf16)
            for tt in range(kc // 128):
                p2r[u, j, c * (kc // 128) + tt] = p[tt * 128:(tt + 1) * 128, :].T.astype(bf16)

        def b_part(t):
            u, j, c = items[t]
            r = _dot(_bf(vT32[:, c * kc:(c + 1) * kc]), _bf(pr[u, j, c * kc // 2:(c + 1) * kc // 2, :]))
            acc[(u, j)] = r if c == 0 else acc[(u, j)] + r
            if c == nc - 1:
                l = jnp.sum(lsum[(u, j)], axis=0, keepdims=True)
                linv = 1.0 / l
                oT_s[j, pl.ds(r0(u), 16), :] = acc[(u, j)] * linv
                l_s[j, pl.ds(h0 + u, 1), :] = l

        for t in range(n + L):
            if t < n:
                a_part(t)
            if t - L >= 0:
                b_part(t - L)
        return carry

    def true_max(h, carry):
        rr = pl.multiple_of(h * 32, 32)
        for j in range(NJ):
            qh = qa_s[j, pl.ds(rr, 32), :].astype(f32)
            row = lax.broadcasted_iota(jnp.int32, (32, W), 0)
            qh = jnp.where(row < DH, qh, 0.0).astype(bf16)
            m = None
            for c in range(S // 256):
                s = _dot(ka_s[c * 256:(c + 1) * 256, :], qh)
                mc = jnp.max(s, axis=0, keepdims=True)
                m = mc if m is None else jnp.maximum(m, mc)
            ext = _split3_rows(-m.reshape(1, 1, W), 1, W).reshape(16, W)
            qa_s[j, pl.ds(pl.multiple_of(rr + 16, 16), 16), :] = ext.astype(bf16)
        return carry

    flag_s[0] = 0

    def attempt(it, carry):
        @pl.when(jnp.logical_or(it == 0, flag_s[0] == 1))
        def _():
            @pl.when(it == 1)
            def _():
                lax.fori_loop(0, H, true_max, 0)
            lax.fori_loop(0, H // FWD_U, fwd_group, 0)
            lmin = jnp.min(jnp.minimum(l_s[0], l_s[1]))
            flag_s[0] = jnp.where(lmin >= SAFE_L, 0, 1).astype(jnp.int32)
        return carry

    lax.fori_loop(0, 2, attempt, 0)

    @pl.when(i == 0)
    def _weights():
        wo_copy.wait()
        woT_s[...] = _tr(wo_ref[...])
        w1_copy.wait()
        w1_s[...] = _tr(w1T_ref[...])
        w3_copy.wait()
        w3_s[...] = _tr(w3T_ref[...])
        w2_copy.wait()
        w2T_s[...] = _tr(w2_ref[...])

    def acc(ref, val):
        ref[...] = jnp.where(i == 0, 0.0, ref[...]) + val

    g = g_ref[...]
    dact = _dot_nt(w2_ref[...], g)
    oT = jnp.concatenate([oT_s[j] for j in range(NJ)], axis=1)
    oTb = oT.astype(bf16)
    hT = x_ref[cols, :].astype(f32).T + _dot(woT_s[...], oTb)
    hhat, hrstd = _lnT_fwd(hT)
    hnT = hhat.astype(bf16)
    gate = _dot(w1T_ref[...], hnT)
    up = _dot(w3T_ref[...], hnT)
    sig = 0.5 * jnp.tanh(0.5 * gate) + 0.5
    silu = gate * sig
    act = (silu * up).astype(bf16)
    out_ref[...] = (hT + _dot(w2T_s[...], act)).T.astype(out_ref.dtype)

    gT = g.astype(f32).T
    dup = (dact * silu).astype(bf16)
    dgate = (dact * up * (sig * (1.0 + gate * (1.0 - sig)))).astype(bf16)
    acc(a_w1T, _dot_nt(dgate, hnT))
    acc(a_w3T, _dot_nt(dup, hnT))
    dhn = _dot(w1_s[...], dgate) + _dot(w3_s[...], dup)
    dhT = gT + _lnT_bwd(dhn, hhat, hrstd)
    dhT_s[:, cols] = dhT
    dhb = dhT.astype(bf16)
    acc(a_wo, _dot_nt(oTb, dhb))
    doT = _dot(wo_ref[...], dhb)

    linv = 1.0 / jnp.concatenate([l_s[j] for j in range(NJ)], axis=1)
    do3 = doT.reshape(H, DH, BQ)
    delta = jnp.sum(do3 * oT.reshape(H, DH, BQ), axis=1, keepdims=True)
    linv3 = linv.reshape(H, 1, BQ)
    doa = jnp.concatenate([do3 * linv3, _split3_rows(-delta * linv3, H, BQ)], axis=1)
    doa = doa.reshape(2 * D, BQ).astype(bf16)
    for j in range(NJ):
        doa_s[j] = doa[:, j * W:(j + 1) * W]
    acc(a_w2, _dot(act, g))

    dw1_copy = pltpu.make_async_copy(w1T_ref, dw1T_hbm, out_sem.at[0])
    dw3_copy = pltpu.make_async_copy(w3T_ref, dw3T_hbm, out_sem.at[1])
    dw2_copy = pltpu.make_async_copy(w2_ref, dw2_hbm, out_sem.at[2])
    dwo_copy = pltpu.make_async_copy(wo_ref, dwo_hbm, out_sem.at[3])

    @pl.when(i == NB - 1)
    def _early_out():
        w1T_ref[...] = a_w1T[...].astype(bf16)
        dw1_copy.start()
        w3T_ref[...] = a_w3T[...].astype(bf16)
        dw3_copy.start()
        w2_ref[...] = a_w2[...].astype(bf16)
        dw2_copy.start()
        wo_ref[...] = a_wo[...].astype(bf16)
        dwo_copy.start()

    def bwd_group(gi, carry):
        kc, U = BWD_KC, BWD_U
        nc = S // kc
        h0 = gi * U
        pr = p32.at[pl.ds(h0, U)]
        p2r = p2_32.at[pl.ds(h0, U)]
        items = [(u, j, c) for u in range(U) for j in range(NJ) for c in range(nc)]
        n = len(items)
        dsv, dq = {}, {}

        def r0(u):
            return pl.multiple_of((h0 + u) * 16, 16)

        def d_part(t):
            u, j, c = items[t]
            do_aug = _bf(doa32[j, pl.ds(r0(u), 16), :])
            dp = _dot(_bf(va32[c * kc // 2:(c + 1) * kc // 2, :]), do_aug)
            pc = _bf(pr[u, j, c * kc // 2:(c + 1) * kc // 2, :])
            dsv[t] = (pc.astype(f32) * dp).astype(bf16)

        def e_part(t):
            u, j, c = items[t]
            do16 = _bf(doa32[j, pl.ds(r0(u), 8), :])
            assert kc == 128
            dvT_s[:, c * kc:(c + 1) * kc] += _dot(do16, _bf(p2r[u, j, c]))

        def f_part(t):
            u, j, c = items[t]
            r = _dot(_bf(kT32[:, c * kc:(c + 1) * kc]), dsv[t])
            dq[(u, j)] = r if c == 0 else dq[(u, j)] + r
            if c == nc - 1:
                dqT_s[j, pl.ds(r0(u), 16), :] = dq[(u, j)]

        def g_part(t):
            u, j, c = items[t]
            q16 = _bf(qa32[j, pl.ds(r0(u), 8), :])
            dkT_s[:, c * kc:(c + 1) * kc] += _dot_nt(q16, dsv[t])

        parts = {"d": (d_part, 0), "e": (e_part, BWD_LE), "f": (f_part, BWD_LF), "g": (g_part, BWD_LG)}
        order = ["defg", "dfeg", "dgfe", "edfg", "dgef", "fdge", "gdfe", "degf"][BWD_ORD]
        for t in range(n + max(BWD_LE, BWD_LF, BWD_LG)):
            for ch in order:
                fn, lag = parts[ch]
                if 0 <= t - lag < n:
                    fn(t - lag)
        return carry

    lax.fori_loop(0, H // BWD_U, bwd_group, 0)

    dqT = (jnp.concatenate([dqT_s[j] for j in range(NJ)], axis=1) * (DH ** -0.5)).astype(bf16)
    acc(a_wq, _dot_nt(xnT, dqT))
    dxnT_s[:, cols] = _dot(wq_ref[...], dqT)

    @pl.when(i == NB - 1)
    def _epilogue():
        wq_ref[...] = a_wq[...].astype(bf16)
        dwq_copy = pltpu.make_async_copy(wq_ref, dwq_hbm, out_sem.at[4])
        dwq_copy.start()
        wkv = jnp.concatenate([wkv_ref[...].astype(f32), jnp.zeros((128 - 2 * DH, D), f32)], axis=0)
        wkv = wkv.T[:, 0:2 * DH].astype(bf16)

        dkvT = jnp.concatenate([dkT_s[...] * LN2, dvT_s[...]], axis=0).astype(bf16)
        dwkv_s[...] = _dot_nt(dkvT, xnT_s[...]).astype(bf16)
        dwk_copy = pltpu.make_async_copy(dwkv_s.at[0:DH, :], dwkT_hbm, out_sem.at[5])
        dwv_copy = pltpu.make_async_copy(dwkv_s.at[DH:2 * DH, :], dwvT_hbm, out_sem.at[6])
        dwk_copy.start()
        dwv_copy.start()

        def dx_copy(b):
            cs = pl.ds(pl.multiple_of(b * BQ, BQ), BQ)
            return pltpu.make_async_copy(x_ref.at[cs, :], dx_hbm.at[cs, :], out_sem.at[7 + b])

        def blk(b, carry):
            cs = pl.ds(pl.multiple_of(b * BQ, BQ), BQ)
            xhat = xnT_s[:, cs].astype(f32)
            rstd = rstd_s[:, cs]
            dkv = jnp.concatenate([dkT_s[:, cs] * LN2, dvT_s[:, cs]], axis=0)
            dxn = dxnT_s[:, cs] + _dot(wkv, dkv.astype(bf16))
            dxT = dhT_s[:, cs] + _lnT_bwd(dxn, xhat, rstd)
            x_ref[cs, :] = dxT.T.astype(bf16)
            dx_copy(b).start()
            return carry

        lax.fori_loop(0, NB // 2, lambda b, c: blk(2 * b + 1, blk(2 * b, c)), 0)
        dw1_copy.wait()
        dw3_copy.wait()
        dw2_copy.wait()
        dwo_copy.wait()
        dwq_copy.wait()
        for b in range(NB):
            dx_copy(b).wait()
        dwk_copy.wait()
        dwv_copy.wait()


def _const(shape):
    nd = len(shape)
    return pl.BlockSpec(shape, lambda i: (0,) * nd, pipeline_mode=pl.Buffered(1))


@jax.jit
def pallas_sequential_preLN__grouped_kv_mqa__glu_gated_swiglu__prompt_kernel(A_x, A_wq, A_wk, A_wv, A_wo, B_x, B_w1, B_w3, B_w2, grad_out):
    del B_x
    x = A_x.reshape(S, D)
    g = grad_out.reshape(S, D)
    out_shape = [
        jax.ShapeDtypeStruct((S, D), bf16),
        jax.ShapeDtypeStruct((S, D), bf16),
        jax.ShapeDtypeStruct((D, D), bf16),
        jax.ShapeDtypeStruct((DH, D), bf16),
        jax.ShapeDtypeStruct((DH, D), bf16),
        jax.ShapeDtypeStruct((D, D), bf16),
        jax.ShapeDtypeStruct((F, D), bf16),
        jax.ShapeDtypeStruct((F, D), bf16),
        jax.ShapeDtypeStruct((F, D), bf16),
    ]
    hbm = pl.BlockSpec(memory_space=pl.ANY)
    in_specs = [hbm] * 8 + [pl.BlockSpec((BQ, D), lambda i: (i, 0))]
    out_specs = [pl.BlockSpec((BQ, D), lambda i: (i, 0))] + [hbm] * 8
    scratch = [
        pltpu.VMEM((S, D), bf16),
        pltpu.VMEM((D, D), bf16),
        pltpu.VMEM((2 * DH, D), bf16),
        pltpu.VMEM((D, D), bf16),
        pltpu.VMEM((F, D), bf16),
        pltpu.VMEM((F, D), bf16),
        pltpu.VMEM((F, D), bf16),
        pltpu.VMEM((2 * DH, D), bf16),
        pltpu.SemaphoreType.DMA((NB + 7,)),
        pltpu.SemaphoreType.DMA((NB + 7,)),
        pltpu.VMEM((1, S), f32),
        pltpu.VMEM((D, S), bf16),
        pltpu.VMEM((D, D), bf16),
        pltpu.VMEM((D, D), bf16),
        pltpu.VMEM((D, F), bf16),
        pltpu.VMEM((D, F), bf16),
        pltpu.VMEM((D, F), bf16),
        pltpu.VMEM((S, 32), bf16),
        pltpu.VMEM((S, 32), bf16),
        pltpu.VMEM((DH, S), bf16),
        pltpu.VMEM((DH, S), bf16),
        pltpu.VMEM((8, BQ), f32),
        pltpu.VMEM((NJ, 2 * D, W), bf16),
        pltpu.VMEM((NJ, 2 * D, W), bf16),
        pltpu.VMEM((H, NJ, S, W), bf16),
        pltpu.VMEM((H, NJ, S // 128, W, 128), bf16),
        pltpu.VMEM((NJ, D, W), f32),
        pltpu.VMEM((NJ, H, W), f32),
        pltpu.VMEM((NJ, D, W), f32),
        pltpu.VMEM((DH, S), f32),
        pltpu.VMEM((DH, S), f32),
        pltpu.VMEM((D, S), f32),
        pltpu.VMEM((D, S), f32),
        pltpu.VMEM((D, D), f32),
        pltpu.VMEM((D, D), f32),
        pltpu.VMEM((F, D), f32),
        pltpu.VMEM((F, D), f32),
        pltpu.VMEM((F, D), f32),
        pltpu.SMEM((1,), jnp.int32),
    ]
    outs = pl.pallas_call(
        _kernel,
        grid=(NB,),
        in_specs=in_specs,
        out_specs=out_specs,
        out_shape=out_shape,
        scratch_shapes=scratch,
        compiler_params=pltpu.CompilerParams(
            dimension_semantics=("arbitrary",),
            vmem_limit_bytes=120 * 1024 * 1024,
        ),
    )(x, A_wq, A_wk.T, A_wv.T, A_wo, B_w1.T, B_w3.T, B_w2, g)
    h2, dx, dwq, dwkT, dwvT, dwo, dw1T, dw3T, dw2 = outs
    return (h2.reshape(1, S, D), dx.reshape(1, S, D), dwq, dwkT.T, dwvT.T, dwo, dw1T.T, dw3T.T, dw2)
```
